```python
import jax
import jax.numpy as jnp

def _softmax(x, axis=-1):
    return jax.nn.softmax(x, axis=axis)
def _gelu(x):
    return jax.nn.gelu(x, approximate=True)
def _silu(x):
    return jax.nn.silu(x)
def _sigmoid(x):
    return jax.nn.sigmoid(x)
def _layernorm(x, axis=-1, eps=1e-5):
    m = jnp.mean(x, axis=axis, keepdims=True)
    v = jnp.var(x, axis=axis, keepdims=True)
    return (x - m) / jnp.sqrt(v + eps)
def _scatter_add(tgt, idx, src, axis=0):
    return tgt.at[idx].add(src)
def _segment_sum(src, seg, n):
    return jax.ops.segment_sum(src, seg, n)
class _Rng:
    def __init__(self, key):
        self._k = key
    def _next(self):
        self._k, sub = jax.random.split(self._k)
        return sub
    def normal(self, shape):
        return jax.random.normal(self._next(), shape, dtype=jnp.bfloat16)
    def randint(self, lo, hi, shape):
        return jax.random.randint(self._next(), shape, lo, hi, dtype=jnp.int32)
    def uniform(self, shape, lo=0.0, hi=1.0):
        return jax.random.uniform(self._next(), shape, jnp.bfloat16, lo, hi)
    def permutation(self, n):
        return jax.random.permutation(self._next(), n)


kernel_name = 'interleave_layers__sliding_block_cached__dense_activation_gelu__decode'

def _fwd_setup_inputs():
    _rng = _Rng(jax.random.key(int.from_bytes(__import__("os").urandom(4), "little")))
    _w = (lambda a: (lambda t: t.astype(jnp.bfloat16) if jnp.issubdtype(t.dtype, jnp.floating) else t)(jnp.asarray(a)))
    def _A_setup():
        B, Sq, D = 2, 1, 512
        Hq, Hkv, Sk, Dh = 32, 8, 32768, 128
        assert Hq % Hkv == 0, (Hq, Hkv)
        return {
            "x": _w((lambda *s: _rng.normal(s) * 0.05)(B, Sq, D)),
            "k_cache": _w((lambda *s: _rng.normal(s) * 0.05)(B, Hkv, Sk, Dh)),
            "v_cache": _w((lambda *s: _rng.normal(s) * 0.05)(B, Hkv, Sk, Dh)),
            "wq": _w((lambda *s: _rng.normal(s) * 0.05)(D, Hq * Dh) * (D ** -0.5)),
            "wo": _w((lambda *s: _rng.normal(s) * 0.05)(Hq * Dh, D) * ((Hq * Dh) ** -0.5)),
        }
    _A_in = _A_setup()

    def _B_setup():
        B, S, D, F = 2, 1, 512, 1792
        return {
            "x": _w((lambda *s: _rng.normal(s) * 0.05)(B, S, D)),
            "w1": _w((lambda *s: _rng.normal(s) * 0.05)(D, F) * (D ** -0.5)),
            "b1": _w((lambda *s: _rng.normal(s) * 0.05)(F) * 0.01),
            "w2": _w((lambda *s: _rng.normal(s) * 0.05)(F, D) * (F ** -0.5)),
            "b2": _w((lambda *s: _rng.normal(s) * 0.05)(D) * 0.01),
        }
    _B_in = _B_setup()

    return {
        "A_x": _A_in["x"],
        "A_k_cache": _A_in["k_cache"],
        "A_v_cache": _A_in["v_cache"],
        "A_wq": _A_in["wq"],
        "A_wo": _A_in["wo"],
        "B_x": _B_in["x"],
        "B_w1": _B_in["w1"],
        "B_b1": _B_in["b1"],
        "B_w2": _B_in["w2"],
        "B_b2": _B_in["b2"],
    }

def _fwd_reference(A_x, A_k_cache, A_v_cache, A_wq, A_wo, B_x, B_w1, B_b1, B_w2, B_b2):
    def _A_ref(x, k_cache, v_cache, wq, wo):
        B, Sq, D = x.shape
        Hq, Dh = 32, 128
        Hkv, Sk = k_cache.shape[1], k_cache.shape[2]
        W = min(4096, max(256, Sk // 4))
        rep = Hq // Hkv
        q = (lambda x, *d: x.transpose(*d))((x @ wq).reshape(B, Sq, Hq, Dh), 0, 2, 1, 3)
        k = jnp.repeat(k_cache[:, :, Sk - W:, :], rep, axis=1)
        v = jnp.repeat(v_cache[:, :, Sk - W:, :], rep, axis=1)
        scores = jnp.einsum("bhqd,bhkd->bhqk", q, k) * (Dh ** -0.5)
        p = _softmax(scores, axis=-1)
        o = jnp.einsum("bhqk,bhkd->bhqd", p, v)
        return (lambda x, *d: x.transpose(*d))(o, 0, 2, 1, 3).reshape(B, Sq, Hq * Dh) @ wo

    def _B_ref(x, w1, b1, w2, b2):
        h = jnp.einsum("bsd,df->bsf", x, w1) + b1
        h = _gelu(h)
        return jnp.einsum("bsf,fd->bsd", h, w2) + b2

    x = A_x
    x = x + _A_ref(_layernorm(x, axis=-1), A_k_cache, A_v_cache, A_wq, A_wo)
    x = x + _B_ref(_layernorm(x, axis=-1), B_w1, B_b1, B_w2, B_b2)
    x = x + _A_ref(_layernorm(x, axis=-1), A_k_cache, A_v_cache, A_wq, A_wo)
    x = x + _B_ref(_layernorm(x, axis=-1), B_w1, B_b1, B_w2, B_b2)
    return x


def setup_inputs():
    _inp = _fwd_setup_inputs()
    _gk = jax.random.fold_in(jax.random.key(int.from_bytes(__import__("os").urandom(4), "little")), 2**31 - 1)
    _shapes = [[2, 1, 512]]
    _dtypes = ['bfloat16']
    _gks = jax.random.split(_gk, len(_shapes))
    _gs = [jax.random.normal(k, s, dtype=jnp.dtype(d)) * 0.05 for k, s, d in zip(_gks, _shapes, _dtypes)]
    _inp["grad_out"] = _gs[0]
    return _inp

def reference(A_x, A_k_cache, A_v_cache, A_wq, A_wo, B_w1, B_b1, B_w2, B_b2, B_x, grad_out):
    _const = dict(B_x=B_x)
    def _f(*_d):
        return _fwd_reference(**{'A_x': _d[0], 'A_k_cache': _d[1], 'A_v_cache': _d[2], 'A_wq': _d[3], 'A_wo': _d[4], 'B_w1': _d[5], 'B_b1': _d[6], 'B_w2': _d[7], 'B_b2': _d[8], **_const})
    _out, _vjp = jax.vjp(_f, A_x, A_k_cache, A_v_cache, A_wq, A_wo, B_w1, B_b1, B_w2, B_b2)
    _grads = _vjp(grad_out)
    _out0 = jnp.asarray(_out)
    return (_out0, *[jnp.asarray(_g) for _g in _grads])
```

```python
import math

import jax
import jax.numpy as jnp
import jax.experimental.pallas as pl
import jax.experimental.pallas.tpu as pltpu
from jax import lax

_HQ = 32
_LN_EPS = 1e-5
_GELU_C = math.sqrt(2.0 / math.pi)
_GELU_A = 0.044715
_ZERO_ROWS = 128
_GRAD_ROWS = 128
_F32 = jnp.float32
_BF16 = jnp.bfloat16

_NN = (((1,), (0,)), ((), ()))
_NT = (((1,), (1,)), ((), ()))


def _dot(a, b, dims=_NN):
    return lax.dot_general(a, b, dims, preferred_element_type=_F32)


def _layernorm(x):
    mean = jnp.mean(x, axis=-1, keepdims=True)
    xc = x - mean
    var = jnp.mean(xc * xc, axis=-1, keepdims=True)
    rstd = lax.rsqrt(var + _LN_EPS)
    return xc * rstd, rstd


def _layernorm_bwd(dh, h, rstd):
    m1 = jnp.mean(dh, axis=-1, keepdims=True)
    m2 = jnp.mean(dh * h, axis=-1, keepdims=True)
    return rstd * (dh - m1 - h * m2)


def _gelu_and_grad(u):
    u2 = u * u
    t = jnp.tanh(_GELU_C * (u + _GELU_A * u2 * u))
    cdf = 0.5 * (1.0 + t)
    dcdf = 0.5 * (1.0 - t * t) * _GELU_C * (1.0 + 3.0 * _GELU_A * u2)
    return u * cdf, cdf + u * dcdf


def _kernel(
    x_hbm, k_hbm, v_hbm, wq_hbm, wo_hbm, w1_hbm, b1_hbm, w2_hbm, b2_hbm, g_hbm,
    out_hbm, gx_hbm, dk_hbm, dv_hbm, dwq_hbm, dwo_hbm, dw1_hbm, db1_hbm, dw2_hbm,
    db2_hbm,
    x_v, k_v, v_v, wq_v, wo_v, w1_v, b1_v, w2_v, b2_v, g_v,
    out_v, gx_v, dk_v, dv_v, dwq_v, dwo_v, dw1_v, db1_v, dw2_v, db2_v,
    zero_v, p_v, ds_v, pt_v, dst_v, q_v, do_v, res_v,
    in_sem, out_sem,
):
    n_slab, n_part, win, dh = k_hbm.shape
    n_batch = x_hbm.shape[0]
    n_group = n_slab // n_batch
    rep = _HQ // n_group
    rows = n_batch * rep
    last = n_part - 1
    scale = dh ** -0.5

    loads = [
        pltpu.make_async_copy(src, dst, in_sem)
        for src, dst in (
            (k_hbm.at[:, last], k_v), (v_hbm.at[:, last], v_v),
            (wq_hbm, wq_v), (wo_hbm, wo_v), (w1_hbm, w1_v), (w2_hbm, w2_v),
            (x_hbm, x_v), (g_hbm, g_v), (b1_hbm, b1_v), (b2_hbm, b2_v),
        )
    ]
    for i, cp in enumerate(loads):
        cp.start(priority=i % 2)
    zero_v[...] = jnp.zeros(zero_v.shape, zero_v.dtype)
    for cp in loads:
        cp.wait()

    stores = []

    def store(src, dst):
        cp = pltpu.make_async_copy(src, dst, out_sem)
        cp.start()
        stores.append(cp)

    for c in range(win // _ZERO_ROWS):
        for dst in (dk_hbm, dv_hbm):
            store(
                zero_v,
                dst.at[:, pl.ds(0, last), pl.ds(c * _ZERO_ROWS, _ZERO_ROWS)],
            )

    row = lax.broadcasted_iota(jnp.int32, (rows, 1), 0)
    first_batch = row < rep
    head_of_row = row % rep

    def tokens(ref):
        y = ref[...].astype(_F32)
        return jnp.where(first_batch, y[0:1], y[1:2])

    def untokens(y):
        return jnp.concatenate([y[0:1], y[rep:rep + 1]], axis=0)

    def sum_heads(y):
        y0 = jnp.sum(jnp.where(first_batch, y, 0.0), axis=0, keepdims=True)
        y1 = jnp.sum(jnp.where(first_batch, 0.0, y), axis=0, keepdims=True)
        return jnp.where(first_batch, y0, y1)

    def once_per_token(y):
        return jnp.where(head_of_row == 0, y, 0.0)

    def head(y, h):
        return y[:, h * dh:(h + 1) * dh]

    def row_block(g, layer):
        return pl.ds(pl.multiple_of(g * 2 * rows + layer * rows, rows), rows)

    def scatter_heads(y, ref, layer):
        for g in range(n_group):
            t = head(y, g * rep)
            for j in range(1, rep):
                t = jnp.where(head_of_row == j, head(y, g * rep + j), t)
            ref[row_block(g, layer), :] = t

    def gather_heads(ref):
        tiles = []
        for g in range(n_group):
            t = ref[g]
            tiles += [jnp.where(head_of_row == j, t, 0.0) for j in range(rep)]
        return jnp.concatenate(tiles, axis=1)

    def per_batch(lhs, ref, g, dims):
        return jnp.where(
            first_batch, _dot(lhs, ref[g], dims), _dot(lhs, ref[n_group + g], dims)
        )

    def attn_fwd(x, layer):
        h, rstd = _layernorm(x)
        scatter_heads(_dot(h.astype(_BF16), wq_v[...]), q_v, layer)

        def body(g, carry):
            blk = row_block(g, layer)
            s = per_batch(q_v[blk, :].astype(_BF16), k_v, g, _NT) * scale
            e = jnp.exp(s - jnp.max(s, axis=-1, keepdims=True))
            p = e / jnp.sum(e, axis=-1, keepdims=True)
            p_v[blk, :] = p
            res_v[g] = per_batch(p.astype(_BF16), v_v, g, _NN)
            return carry

        lax.fori_loop(0, n_group, body, 0)
        o = gather_heads(res_v)
        return x + sum_heads(_dot(o.astype(_BF16), wo_v[...])), (h, rstd, o)

    def attn_bwd(dy, saved, layer):
        h, rstd, _ = saved
        scatter_heads(_dot(dy.astype(_BF16), wo_v[...], _NT), do_v, layer)

        def body(g, carry):
            blk = row_block(g, layer)
            p = p_v[blk, :]
            dp = per_batch(do_v[blk, :].astype(_BF16), v_v, g, _NT)
            ds = p * (dp - jnp.sum(p * dp, axis=-1, keepdims=True)) * scale
            ds_v[blk, :] = ds
            res_v[g] = per_batch(ds.astype(_BF16), k_v, g, _NN)
            return carry

        lax.fori_loop(0, n_group, body, 0)
        dq = gather_heads(res_v)
        dhid = sum_heads(_dot(dq.astype(_BF16), wq_v[...], _NT))
        return dy + _layernorm_bwd(dhid, h, rstd), dq

    def mlp_fwd(x):
        h, rstd = _layernorm(x)
        u = _dot(h.astype(_BF16), w1_v[...]) + b1_v[...].astype(_F32).reshape(1, -1)
        a, da_du = _gelu_and_grad(u)
        y = _dot(a.astype(_BF16), w2_v[...]) + b2_v[...].astype(_F32).reshape(1, -1)
        return x + y, (h, rstd, a, da_du)

    def mlp_bwd(dy, saved):
        h, rstd, _, da_du = saved
        du = _dot(dy.astype(_BF16), w2_v[...], _NT) * da_du
        dhid = _dot(du.astype(_BF16), w1_v[...], _NT)
        return dy + _layernorm_bwd(dhid, h, rstd), du

    x0 = tokens(x_v)
    x1, sa0 = attn_fwd(x0, 0)
    x2, sm0 = mlp_fwd(x1)
    x3, sa1 = attn_fwd(x2, 1)
    x4, sm1 = mlp_fwd(x3)
    d4 = tokens(g_v)
    d3, du1 = mlp_bwd(d4, sm1)
    d2, dq1 = attn_bwd(d3, sa1, 1)
    d1, du0 = mlp_bwd(d2, sm0)
    d0, dq0 = attn_bwd(d1, sa0, 0)

    out_v[...] = untokens(x4).astype(out_v.dtype)
    gx_v[...] = untokens(d0).astype(gx_v.dtype)
    du = once_per_token(du0), once_per_token(du1)
    dm = once_per_token(d2), once_per_token(d4)
    db1_v[...] = jnp.sum(du[0] + du[1], axis=0).astype(db1_v.dtype)
    db2_v[...] = jnp.sum(dm[0] + dm[1], axis=0).astype(db2_v.dtype)
    for src, dst in ((out_v, out_hbm), (gx_v, gx_hbm), (db1_v, db1_hbm),
                     (db2_v, db2_hbm)):
        store(src, dst)

    def weight_grad(lhs, rhs, ref, dst):
        lhs_t = jnp.concatenate(lhs, axis=0).T.astype(_BF16)
        rhs = jnp.concatenate(rhs, axis=0).astype(_BF16)
        step = 256
        for r in range(0, ref.shape[0], step):
            ref[r:r + step, :] = _dot(lhs_t[r:r + step], rhs).astype(ref.dtype)
        store(ref, dst)

    weight_grad((sa0[0], sa1[0]), (dq0, dq1), dwq_v, dwq_hbm)
    weight_grad((sa0[2], sa1[2]), (d1, d3), dwo_v, dwo_hbm)
    weight_grad((sm0[0], sm1[0]), du, dw1_v, dw1_hbm)
    weight_grad((sm0[2], sm1[2]), dm, dw2_v, dw2_hbm)

    stacked = n_group * 2 * rows
    srow = lax.broadcasted_iota(jnp.int32, (stacked, 1), 0)
    pt_v[...] = p_v[...].T.astype(_BF16)
    dst_v[...] = ds_v[...].T.astype(_BF16)

    def cache_grad(g, carry):
        for left, right, ref in ((dst_v, q_v, dk_v), (pt_v, do_v, dv_v)):
            for b in range(n_batch):
                mine = jnp.logical_and(srow // (2 * rows) == g,
                                       (srow % rows) // rep == b)
                rhs = jnp.where(mine, right[...], 0.0).astype(_BF16)
                ref[b * n_group + g] = _dot(left[...], rhs).astype(ref.dtype)
        return carry

    lax.fori_loop(0, n_group, cache_grad, 0)
    for c in range(win // _GRAD_ROWS):
        part = pl.ds(c * _GRAD_ROWS, _GRAD_ROWS)
        store(dk_v.at[:, part], dk_hbm.at[:, last, part])
        store(dv_v.at[:, part], dv_hbm.at[:, last, part])

    for cp in stores:
        cp.wait()


@jax.jit
def pallas_interleave_layers__sliding_block_cached__dense_activation_gelu__decode_kernel(
    A_x: jax.Array,
    A_k_cache: jax.Array,
    A_v_cache: jax.Array,
    A_wq: jax.Array,
    A_wo: jax.Array,
    B_x: jax.Array,
    B_w1: jax.Array,
    B_b1: jax.Array,
    B_w2: jax.Array,
    B_b2: jax.Array,
    grad_out: jax.Array,
):
    del B_x
    n_batch, n_group, seq, dh = A_k_cache.shape
    win = min(4096, max(256, seq // 4))
    rows = n_batch * (_HQ // n_group)
    assert n_batch == 2 and rows == 8 and seq % win == 0 and dh == 128
    stacked = n_group * 2 * rows

    parts = (n_batch * n_group, seq // win, win, dh)
    window = (n_batch * n_group, win, dh)
    x = A_x.reshape(n_batch, -1)
    inputs = (x, A_k_cache.reshape(parts), A_v_cache.reshape(parts), A_wq, A_wo,
              B_w1, B_b1, B_w2, B_b2, grad_out.reshape(x.shape))
    like = (x, x) + inputs[1:9]

    def staged(arrays):
        return [pltpu.VMEM(window if a.shape == parts else a.shape, a.dtype)
                for a in arrays]

    hbm = pl.BlockSpec(memory_space=pl.ANY)
    res = pl.pallas_call(
        _kernel,
        out_shape=[jax.ShapeDtypeStruct(a.shape, a.dtype) for a in like],
        in_specs=[hbm] * len(inputs),
        out_specs=[hbm] * len(like),
        scratch_shapes=staged(inputs) + staged(like) + [
            pltpu.VMEM((parts[0], parts[1] - 1, _ZERO_ROWS, dh), A_k_cache.dtype),
            pltpu.VMEM((stacked, win), _F32),
            pltpu.VMEM((stacked, win), _F32),
            pltpu.VMEM((win, stacked), _BF16),
            pltpu.VMEM((win, stacked), _BF16),
            pltpu.VMEM((stacked, dh), _F32),
            pltpu.VMEM((stacked, dh), _F32),
            pltpu.VMEM((n_group, rows, dh), _F32),
            pltpu.SemaphoreType.DMA(()),
            pltpu.SemaphoreType.DMA(()),
        ],
        compiler_params=pltpu.CompilerParams(vmem_limit_bytes=112 * 1024 * 1024),
    )(*inputs)
    shaped = (A_x, A_x, A_k_cache, A_v_cache)
    return (*(r.reshape(a.shape) for r, a in zip(res, shaped)), *res[4:])
```

```python
import math

import jax
import jax.numpy as jnp
import jax.experimental.pallas as pl
import jax.experimental.pallas.tpu as pltpu
from jax import lax

_HQ = 32
_LAYERS = 2
_LN_EPS = 1e-5
_GELU_C = math.sqrt(2.0 / math.pi)
_GELU_A = 0.044715

_READ_ROWS, _READ_SLABS = 128, 4
_ZERO_ROWS = 64
_GRAD_ROWS, _GRAD_SLABS = 64, 8
_WEIGHT_STREAMS = 8
_KEYS = 1024
_HIDDEN = 256
_GRAD_KEYS = 128

_F32 = jnp.float32
_BF16 = jnp.bfloat16
_NN = (((1,), (0,)), ((), ()))
_NT = (((1,), (1,)), ((), ()))


def _dot(a, b, dims=_NN):
    return lax.dot_general(a, b, dims, preferred_element_type=_F32)


def _block(i, size):
    return pl.ds(pl.multiple_of(i * size, size), size)


def _loop(n, body):
    lax.fori_loop(0, n, lambda i, carry: (body(i), carry)[1], 0)


def _layernorm(x):
    xc = x - jnp.mean(x, axis=-1, keepdims=True)
    rstd = lax.rsqrt(jnp.mean(xc * xc, axis=-1, keepdims=True) + _LN_EPS)
    return xc * rstd, rstd


def _layernorm_bwd(dh, h, rstd):
    m1 = jnp.mean(dh, axis=-1, keepdims=True)
    m2 = jnp.mean(dh * h, axis=-1, keepdims=True)
    return rstd * (dh - m1 - h * m2)


def _gelu_and_grad(u):
    u2 = u * u
    t = jnp.tanh(_GELU_C * (u + _GELU_A * u2 * u))
    cdf = 0.5 * (1.0 + t)
    dcdf = 0.5 * (1.0 - t * t) * _GELU_C * (1.0 + 3.0 * _GELU_A * u2)
    return u * cdf, cdf + u * dcdf


def _fold_lanes(y, op):
    acc = y[:, :128]
    for t in range(128, y.shape[1], 128):
        acc = op(acc, y[:, t:t + 128])
    return acc


def _kernel(
    x_hbm, k_hbm, v_hbm, wq_hbm, wo_hbm, w1_hbm, b1_hbm, w2_hbm, b2_hbm, g_hbm,
    out_hbm, gx_hbm, dk_hbm, dv_hbm, dwq_hbm, dwo_hbm, dw1_hbm, db1_hbm, dw2_hbm,
    db2_hbm,
    x_v, k_v, v_v, wq_v, wo_v, w1_v, b1_v, w2_v, b2_v, g_v,
    out_v, gx_v, dk_v, dv_v, dwq_v, dwo_v, dw1_v, db1_v, dw2_v, db2_v,
    zero_v, p_v, ds_v, q_v, do_v, qm_v, dom_v,
    ha_v, hm_v, ra_v, rm_v, o_v, dq_v, dya_v, dym_v, a_v, dadu_v, du_v, bias_v,
    k_sem, v_sem, in_sem, late_sem, dk_sem, dv_sem, out_sem, dw_sem,
):
    n_slab, n_part, win, dh = k_hbm.shape
    n_batch, d_model = x_hbm.shape
    d_ff = w1_hbm.shape[1]
    n_group = n_slab // n_batch
    rep = _HQ // n_group
    rows = n_batch * rep
    last = n_part - 1
    scale = dh ** -0.5

    def load_window(i):
        slabs = _block(i // (win // _READ_ROWS), _READ_SLABS)
        keys = _block(i % (win // _READ_ROWS), _READ_ROWS)
        pltpu.make_async_copy(
            k_hbm.at[slabs, last, keys], k_v.at[slabs, keys], k_sem
        ).start(priority=0)
        pltpu.make_async_copy(
            v_hbm.at[slabs, last, keys], v_v.at[slabs, keys], v_sem
        ).start(priority=1)

    _loop((n_slab // _READ_SLABS) * (win // _READ_ROWS), load_window)
    cut1, cut2 = d_model * 13 // 16, d_ff * 13 // 16
    head1, tail1 = pl.ds(0, cut1), pl.ds(cut1, d_model - cut1)
    head2, tail2 = pl.ds(0, cut2), pl.ds(cut2, d_ff - cut2)
    loads = [
        pltpu.make_async_copy(src, dst, in_sem)
        for src, dst in (
            (wq_hbm, wq_v), (wo_hbm, wo_v), (x_hbm, x_v), (g_hbm, g_v),
            (b1_hbm, b1_v), (b2_hbm, b2_v),
            (w1_hbm.at[head1], w1_v.at[head1]), (w2_hbm.at[head2], w2_v.at[head2]),
        )
    ]
    late_loads = [
        pltpu.make_async_copy(w1_hbm.at[tail1], w1_v.at[tail1], late_sem),
        pltpu.make_async_copy(w2_hbm.at[tail2], w2_v.at[tail2], late_sem),
    ]
    for i, cp in enumerate(loads + late_loads):
        cp.start(priority=i % 2)
    zero_v[...] = jnp.zeros(zero_v.shape, zero_v.dtype)
    pltpu.make_async_copy(k_v, k_v, k_sem).wait()
    pltpu.make_async_copy(v_v, v_v, v_sem).wait()
    for cp in loads:
        cp.wait()

    per_slab = win // _ZERO_ROWS

    def zero_fill(dst, sem, first, count):
        def start(i):
            i = first + i
            keys = _block(i % per_slab, _ZERO_ROWS)
            pltpu.make_async_copy(
                zero_v, dst.at[i // per_slab, pl.ds(0, last), keys], sem
            ).start()

        _loop(count, start)

    step_fill = n_slab * per_slab // (2 * _LAYERS * n_group)
    zero_fill(dv_hbm, dv_sem, 0, per_slab)
    for cp in late_loads:
        cp.wait()

    row = lax.broadcasted_iota(jnp.int32, (rows, 1), 0)
    first_batch = row < rep
    head_of_row = row % rep

    def tokens(ref):
        y = ref[...].astype(_F32)
        return jnp.where(first_batch, y[0:1], y[1:2])

    def untokens(y):
        return jnp.concatenate([y[0:1], y[rep:rep + 1]], axis=0)

    def sum_heads(y):
        y0 = jnp.sum(jnp.where(first_batch, y, 0.0), axis=0, keepdims=True)
        y1 = jnp.sum(jnp.where(first_batch, 0.0, y), axis=0, keepdims=True)
        return jnp.where(first_batch, y0, y1)

    def once_per_token(y):
        return jnp.where(head_of_row == 0, y, 0.0)

    def own_head(y):
        t = y[:, :dh]
        for j in range(1, rep):
            t = jnp.where(head_of_row == j, y[:, j * dh:(j + 1) * dh], t)
        return t

    def spread_heads(t):
        return jnp.concatenate(
            [jnp.where(head_of_row == j, t, 0.0) for j in range(rep)], axis=1
        )

    def per_batch(lhs, ref, g, keys, dims):
        lhs = lhs.astype(_BF16)
        return jnp.where(
            first_batch,
            _dot(lhs, ref[g, keys, :], dims),
            _dot(lhs, ref[n_group + g, keys, :], dims),
        )

    zero_tile = jnp.zeros((rows, dh), _F32)
    zero_token = jnp.zeros((rows, d_model), _F32)
    bias_v[...] = jnp.broadcast_to(
        b1_v[...].astype(_F32).reshape(1, d_ff), bias_v.shape
    )

    def attn_fwd(x, layer):
        saved = _block(layer, rows)
        h, rstd = _layernorm(x)
        ha_v[saved, :] = h
        ra_v[saved, :] = jnp.broadcast_to(rstd, (rows, dh))
        hb = h.astype(_BF16)

        def group(g, y):
            zero_fill(dk_hbm, dk_sem, (layer * n_group + g) * step_fill, step_fill)
            heads = _block(g, rep * dh)
            blk = _block(g * _LAYERS + layer, rows)
            q = own_head(_dot(hb, wq_v[:, heads]))
            q_v[blk, :] = q

            def scores(c, m):
                keys = _block(c, _KEYS)
                s = per_batch(q, k_v, g, keys, _NT) * scale
                p_v[blk, keys] = s
                return jnp.maximum(m, _fold_lanes(s, jnp.maximum))

            m = lax.fori_loop(0, win // _KEYS, scores, zero_tile - jnp.inf)
            m = jnp.max(m, axis=-1, keepdims=True)
            e = jnp.exp(p_v[blk, :] - m)
            p_v[blk, :] = e / jnp.sum(e, axis=-1, keepdims=True)

            def values(c, o):
                keys = _block(c, _KEYS)
                return o + per_batch(p_v[blk, keys], v_v, g, keys, _NN)

            o = spread_heads(lax.fori_loop(0, win // _KEYS, values, zero_tile))
            o_v[saved, heads] = o
            return y + _dot(o.astype(_BF16), wo_v[heads, :])

        return x + sum_heads(lax.fori_loop(0, n_group, group, zero_token))

    def attn_bwd(dy, layer):
        saved = _block(layer, rows)
        dya_v[saved, :] = dy
        dyb = dy.astype(_BF16)

        def group(g, dhid):
            done = (_LAYERS + layer) * n_group + g
            zero_fill(dk_hbm, dk_sem, done * step_fill, step_fill)
            heads = _block(g, rep * dh)
            blk = _block(g * _LAYERS + layer, rows)
            do = own_head(_dot(dyb, wo_v[heads, :], _NT))
            do_v[blk, :] = do

            def probs(c, acc):
                keys = _block(c, _KEYS)
                dp = per_batch(do, v_v, g, keys, _NT)
                ds_v[blk, keys] = dp
                return acc + _fold_lanes(dp * p_v[blk, keys], jnp.add)

            delta = lax.fori_loop(0, win // _KEYS, probs, zero_tile)
            delta = jnp.sum(delta, axis=-1, keepdims=True)

            def queries(c, dq):
                keys = _block(c, _KEYS)
                ds = p_v[blk, keys] * (ds_v[blk, keys] - delta) * scale
                ds_v[blk, keys] = ds
                return dq + per_batch(ds, k_v, g, keys, _NN)

            dq = spread_heads(lax.fori_loop(0, win // _KEYS, queries, zero_tile))
            dq_v[saved, heads] = dq
            return dhid + _dot(dq.astype(_BF16), wq_v[:, heads], _NT)

        dhid = sum_heads(lax.fori_loop(0, n_group, group, zero_token))
        return dy + _layernorm_bwd(dhid, ha_v[saved, :], ra_v[saved, 0:1])

    def mlp_fwd(x, layer):
        saved = _block(layer, rows)
        h, rstd = _layernorm(x)
        hm_v[saved, :] = h
        rm_v[saved, :] = jnp.broadcast_to(rstd, (rows, dh))
        hb = h.astype(_BF16)

        def step(c, y):
            units = _block(c, _HIDDEN)
            a, da_du = _gelu_and_grad(_dot(hb, w1_v[:, units]) + bias_v[:, units])
            a_v[saved, units] = a
            dadu_v[saved, units] = da_du
            return y + _dot(a.astype(_BF16), w2_v[units, :])

        y = lax.fori_loop(0, d_ff // _HIDDEN, step, zero_token)
        return x + y + b2_v[...].astype(_F32).reshape(1, d_model)

    def mlp_bwd(dy, layer):
        saved = _block(layer, rows)
        dym_v[saved, :] = once_per_token(dy)
        dyb = dy.astype(_BF16)

        def step(c, dhid):
            units = _block(c, _HIDDEN)
            du = _dot(dyb, w2_v[units, :], _NT) * dadu_v[saved, units]
            du_v[saved, units] = once_per_token(du)
            return dhid + _dot(du.astype(_BF16), w1_v[:, units], _NT)

        dhid = lax.fori_loop(0, d_ff // _HIDDEN, step, zero_token)
        return dy + _layernorm_bwd(dhid, hm_v[saved, :], rm_v[saved, 0:1])

    def forward(layer, x):
        return mlp_fwd(attn_fwd(x, layer), layer)

    def backward(i, dy):
        layer = _LAYERS - 1 - i
        return attn_bwd(mlp_bwd(dy, layer), layer)

    out = lax.fori_loop(0, _LAYERS, forward, tokens(x_v))
    gx = lax.fori_loop(0, _LAYERS, backward, tokens(g_v))
    out_v[...] = untokens(out).astype(out_v.dtype)
    gx_v[...] = untokens(gx).astype(gx_v.dtype)
    db1_v[...] = jnp.sum(du_v[...], axis=0).astype(db1_v.dtype)
    db2_v[...] = jnp.sum(dym_v[...], axis=0).astype(db2_v.dtype)

    def weight_grad(lhs, rhs, ref, tile_rows, tile_cols):
        n_col = ref.shape[1] // tile_cols

        def tile(i):
            r, c = _block(i // n_col, tile_rows), _block(i % n_col, tile_cols)
            ref[r, c] = _dot(
                lhs[:, r].T.astype(_BF16), rhs[:, c].astype(_BF16)
            ).astype(ref.dtype)

        _loop((ref.shape[0] // tile_rows) * n_col, tile)

    weights = (
        (ha_v, dq_v, dwq_v, 128, 2048),
        (o_v, dya_v, dwo_v, 512, d_model),
        (hm_v, du_v, dw1_v, 128, d_ff),
        (a_v, dym_v, dw2_v, _HIDDEN, d_model),
    )
    for i, operands in enumerate(weights):
        zero_fill(dv_hbm, dv_sem, (1 + i) * per_slab, per_slab)
        weight_grad(*operands)

    srow = lax.broadcasted_iota(jnp.int32, (q_v.shape[0], 1), 0)
    slab_of_row = (srow % rows) // rep * n_group + srow // (_LAYERS * rows)

    def mask_slab(s):
        for src, dst in ((q_v, qm_v), (do_v, dom_v)):
            dst[:, _block(s, dh)] = jnp.where(
                slab_of_row == s, src[...], 0.0
            ).astype(dst.dtype)

    _loop(n_slab, mask_slab)
    n_step = win // _GRAD_KEYS
    filled = (1 + len(weights)) * per_slab
    grad_fill = (n_slab // 2) * per_slab // n_step

    def cache_grad(c):
        zero_fill(dv_hbm, dv_sem, filled + c * grad_fill, grad_fill)
        keys = _block(c, _GRAD_KEYS)
        for lhs, rhs, ref in ((ds_v, qm_v, dk_v), (p_v, dom_v, dv_v)):
            res = _dot(lhs[:, keys].T.astype(_BF16), rhs[...])
            for s in range(n_slab):
                ref[s, keys, :] = res[:, s * dh:(s + 1) * dh].astype(ref.dtype)

    _loop(n_step, cache_grad)
    filled += n_step * grad_fill
    zero_fill(dv_hbm, dv_sem, filled, n_slab * per_slab - filled)

    def store_window(src, dst, sem):
        def start(i):
            slabs = _block(i // (win // _GRAD_ROWS), _GRAD_SLABS)
            keys = _block(i % (win // _GRAD_ROWS), _GRAD_ROWS)
            pltpu.make_async_copy(
                src.at[slabs, keys], dst.at[slabs, last, keys], sem
            ).start()

        _loop((n_slab // _GRAD_SLABS) * (win // _GRAD_ROWS), start)

    def store_weight(src, dst, sem):
        n_row, n_col = src.shape[0] // _WEIGHT_STREAMS, src.shape[1]
        width = max(w for w in range(128, 513, 128) if n_col % w == 0)
        src = src.reshape(_WEIGHT_STREAMS, n_row, n_col)
        dst = dst.reshape(_WEIGHT_STREAMS, n_row, n_col)

        def start(i):
            r, c = _block(i // (n_col // width), 16), _block(i % (n_col // width), width)
            pltpu.make_async_copy(src.at[:, r, c], dst.at[:, r, c], sem).start()

        _loop((n_row // 16) * (n_col // width), start)

    small = [
        pltpu.make_async_copy(src, dst, out_sem)
        for src, dst in ((out_v, out_hbm), (gx_v, gx_hbm), (db1_v, db1_hbm),
                         (db2_v, db2_hbm))
    ]
    large = ((dwq_v, dwq_hbm), (dwo_v, dwo_hbm), (dw1_v, dw1_hbm),
             (dw2_v, dw2_hbm))
    for cp in small:
        cp.start()
    for i, (src, dst) in enumerate(large):
        store_weight(src, dst, dw_sem.at[i])
    store_window(dk_v, dk_hbm, dk_sem)
    store_window(dv_v, dv_hbm, dv_sem)

    for cp in small:
        cp.wait()
    for i, (src, dst) in enumerate(large):
        pltpu.make_async_copy(src, dst, dw_sem.at[i]).wait()
    pltpu.make_async_copy(dk_hbm, dk_hbm, dk_sem).wait()
    pltpu.make_async_copy(dv_hbm, dv_hbm, dv_sem).wait()


@jax.jit
def pallas_interleave_layers__sliding_block_cached__dense_activation_gelu__decode_kernel(
    A_x: jax.Array,
    A_k_cache: jax.Array,
    A_v_cache: jax.Array,
    A_wq: jax.Array,
    A_wo: jax.Array,
    B_x: jax.Array,
    B_w1: jax.Array,
    B_b1: jax.Array,
    B_w2: jax.Array,
    B_b2: jax.Array,
    grad_out: jax.Array,
):
    del B_x
    n_batch, n_group, seq, dh = A_k_cache.shape
    d_model, d_ff = B_w1.shape
    win = min(4096, max(256, seq // 4))
    rows = n_batch * (_HQ // n_group)
    assert n_batch == 2 and rows == 8 and dh == 128 and seq % win == 0
    n_slab = n_batch * n_group
    stacked = n_group * _LAYERS * rows
    saved = _LAYERS * rows

    parts = (n_slab, seq // win, win, dh)
    x = A_x.reshape(n_batch, d_model)
    inputs = (x, A_k_cache.reshape(parts), A_v_cache.reshape(parts), A_wq, A_wo,
              B_w1, B_b1, B_w2, B_b2, grad_out.reshape(x.shape))
    like = (x, x) + inputs[1:9]

    def staged(arrays):
        return [pltpu.VMEM((n_slab, win, dh) if a.shape == parts else a.shape, a.dtype)
                for a in arrays]

    hbm = pl.BlockSpec(memory_space=pl.ANY)
    res = pl.pallas_call(
        _kernel,
        out_shape=[jax.ShapeDtypeStruct(a.shape, a.dtype) for a in like],
        in_specs=[hbm] * len(inputs),
        out_specs=[hbm] * len(like),
        scratch_shapes=staged(inputs) + staged(like) + [
            pltpu.VMEM((parts[1] - 1, _ZERO_ROWS, dh), A_k_cache.dtype),
            pltpu.VMEM((stacked, win), _F32),
            pltpu.VMEM((stacked, win), _F32),
            pltpu.VMEM((stacked, dh), _F32),
            pltpu.VMEM((stacked, dh), _F32),
            pltpu.VMEM((stacked, n_slab * dh), _BF16),
            pltpu.VMEM((stacked, n_slab * dh), _BF16),
            pltpu.VMEM((saved, d_model), _F32),
            pltpu.VMEM((saved, d_model), _F32),
            pltpu.VMEM((saved, dh), _F32),
            pltpu.VMEM((saved, dh), _F32),
            pltpu.VMEM((saved, _HQ * dh), _F32),
            pltpu.VMEM((saved, _HQ * dh), _F32),
            pltpu.VMEM((saved, d_model), _F32),
            pltpu.VMEM((saved, d_model), _F32),
            pltpu.VMEM((saved, d_ff), _F32),
            pltpu.VMEM((saved, d_ff), _F32),
            pltpu.VMEM((saved, d_ff), _F32),
            pltpu.VMEM((rows, d_ff), _F32),
        ] + [pltpu.SemaphoreType.DMA(())] * 7 + [pltpu.SemaphoreType.DMA((4,))],
        compiler_params=pltpu.CompilerParams(vmem_limit_bytes=112 * 1024 * 1024),
    )(*inputs)
    shaped = (A_x, A_x, A_k_cache, A_v_cache)
    return (*(r.reshape(a.shape) for r, a in zip(res, shaped)), *res[4:])
```

```python
import math

import jax
import jax.numpy as jnp
import jax.experimental.pallas as pl
import jax.experimental.pallas.tpu as pltpu
from jax import lax

_HQ = 32
_LAYERS = 2
_LN_EPS = 1e-5
_GELU_C = math.sqrt(2.0 / math.pi)
_GELU_A = 0.044715

_READ_ROWS, _READ_SLABS = 128, 4
_ZERO_ROWS = 64
_GRAD_ROWS, _GRAD_SLABS = 64, 8
_WEIGHT_STREAMS = 8
_KEYS = 1024
_HIDDEN = 256
_GRAD_KEYS = 128

_F32 = jnp.float32
_BF16 = jnp.bfloat16
_NN = (((1,), (0,)), ((), ()))
_NT = (((1,), (1,)), ((), ()))


def _dot(a, b, dims=_NN):
    return lax.dot_general(a, b, dims, preferred_element_type=_F32)


def _block(i, size):
    return pl.ds(pl.multiple_of(i * size, size), size)


def _loop(n, body):
    lax.fori_loop(0, n, lambda i, carry: (body(i), carry)[1], 0)


def _layernorm(x):
    xc = x - jnp.mean(x, axis=-1, keepdims=True)
    rstd = lax.rsqrt(jnp.mean(xc * xc, axis=-1, keepdims=True) + _LN_EPS)
    return xc * rstd, rstd


def _layernorm_bwd(dh, h, rstd):
    m1 = jnp.mean(dh, axis=-1, keepdims=True)
    m2 = jnp.mean(dh * h, axis=-1, keepdims=True)
    return rstd * (dh - m1 - h * m2)


def _gelu_and_grad(u):
    u2 = u * u
    t = jnp.tanh(_GELU_C * (u + _GELU_A * u2 * u))
    cdf = 0.5 * (1.0 + t)
    dcdf = 0.5 * (1.0 - t * t) * _GELU_C * (1.0 + 3.0 * _GELU_A * u2)
    return u * cdf, cdf + u * dcdf


def _fold_lanes(y, op):
    acc = y[:, :128]
    for t in range(128, y.shape[1], 128):
        acc = op(acc, y[:, t:t + 128])
    return acc


def _kernel(
    x_hbm, k_hbm, v_hbm, wq_hbm, wo_hbm, w1_hbm, b1_hbm, w2_hbm, b2_hbm, g_hbm,
    out_hbm, gx_hbm, dk_hbm, dv_hbm, dwq_hbm, dwo_hbm, dw1_hbm, db1_hbm, dw2_hbm,
    db2_hbm,
    x_v, k_v, v_v, wq_v, wo_v, w1_v, b1_v, w2_v, b2_v, g_v,
    out_v, gx_v, dk_v, dv_v, dwq_v, dwo_v, dw1_v, db1_v, dw2_v, db2_v,
    zero_v, p_v, ds_v, q_v, do_v, qm_v, dom_v,
    ha_v, hm_v, ra_v, rm_v, o_v, dq_v, dya_v, dym_v, a_v, dadu_v, du_v, bias_v,
    k_sem, v_sem, in_sem, late_sem, dk_sem, dv_sem, out_sem, dw_sem,
):
    n_slab, n_part, win, dh = k_hbm.shape
    n_batch, d_model = x_hbm.shape
    d_ff = w1_hbm.shape[1]
    n_group = n_slab // n_batch
    rep = _HQ // n_group
    rows = n_batch * rep
    last = n_part - 1
    scale = dh ** -0.5

    def load_window(i):
        slabs = _block(i // (win // _READ_ROWS), _READ_SLABS)
        keys = _block(i % (win // _READ_ROWS), _READ_ROWS)
        pltpu.make_async_copy(
            k_hbm.at[slabs, last, keys], k_v.at[slabs, keys], k_sem
        ).start(priority=0)
        pltpu.make_async_copy(
            v_hbm.at[slabs, last, keys], v_v.at[slabs, keys], v_sem
        ).start(priority=1)

    _loop((n_slab // _READ_SLABS) * (win // _READ_ROWS), load_window)
    cut1, cut2 = d_model * 13 // 16, d_ff * 13 // 16
    head1, tail1 = pl.ds(0, cut1), pl.ds(cut1, d_model - cut1)
    head2, tail2 = pl.ds(0, cut2), pl.ds(cut2, d_ff - cut2)
    loads = [
        pltpu.make_async_copy(src, dst, in_sem)
        for src, dst in (
            (wq_hbm, wq_v), (wo_hbm, wo_v), (x_hbm, x_v), (g_hbm, g_v),
            (b1_hbm, b1_v), (b2_hbm, b2_v),
            (w1_hbm.at[head1], w1_v.at[head1]), (w2_hbm.at[head2], w2_v.at[head2]),
        )
    ]
    late_loads = [
        pltpu.make_async_copy(w1_hbm.at[tail1], w1_v.at[tail1], late_sem),
        pltpu.make_async_copy(w2_hbm.at[tail2], w2_v.at[tail2], late_sem),
    ]
    for i, cp in enumerate(loads + late_loads):
        cp.start(priority=i % 2)
    zero_v[...] = jnp.zeros(zero_v.shape, zero_v.dtype)
    pltpu.make_async_copy(k_v, k_v, k_sem).wait()
    pltpu.make_async_copy(v_v, v_v, v_sem).wait()
    for cp in loads:
        cp.wait()

    per_slab = win // _ZERO_ROWS

    def zero_fill(dst, sem, first, count):
        def start(i):
            i = first + i
            keys = _block(i % per_slab, _ZERO_ROWS)
            pltpu.make_async_copy(
                zero_v, dst.at[i // per_slab, pl.ds(0, last), keys], sem
            ).start()

        _loop(count, start)

    step_fill = n_slab * per_slab // (2 * _LAYERS * n_group)
    zero_fill(dv_hbm, dv_sem, 0, per_slab)
    for cp in late_loads:
        cp.wait()

    row = lax.broadcasted_iota(jnp.int32, (rows, 1), 0)
    first_batch = row < rep
    head_of_row = row % rep

    def tokens(ref):
        y = ref[...].astype(_F32)
        return jnp.where(first_batch, y[0:1], y[1:2])

    def untokens(y):
        return jnp.concatenate([y[0:1], y[rep:rep + 1]], axis=0)

    def sum_heads(y):
        y0 = jnp.sum(jnp.where(first_batch, y, 0.0), axis=0, keepdims=True)
        y1 = jnp.sum(jnp.where(first_batch, 0.0, y), axis=0, keepdims=True)
        return jnp.where(first_batch, y0, y1)

    def once_per_token(y):
        return jnp.where(head_of_row == 0, y, 0.0)

    def own_head(y):
        t = y[:, :dh]
        for j in range(1, rep):
            t = jnp.where(head_of_row == j, y[:, j * dh:(j + 1) * dh], t)
        return t

    def spread_heads(t):
        return jnp.concatenate(
            [jnp.where(head_of_row == j, t, 0.0) for j in range(rep)], axis=1
        )

    def per_batch(lhs, ref, g, keys, dims):
        lhs = lhs.astype(_BF16)
        return jnp.where(
            first_batch,
            _dot(lhs, ref[g, keys, :], dims),
            _dot(lhs, ref[n_group + g, keys, :], dims),
        )

    zero_tile = jnp.zeros((rows, dh), _F32)
    zero_token = jnp.zeros((rows, d_model), _F32)
    bias_v[...] = jnp.broadcast_to(
        b1_v[...].astype(_F32).reshape(1, d_ff), bias_v.shape
    )

    def attn_fwd(x, layer):
        saved = _block(layer, rows)
        h, rstd = _layernorm(x)
        ha_v[saved, :] = h
        ra_v[saved, :] = jnp.broadcast_to(rstd, (rows, dh))
        hb = h.astype(_BF16)

        def group(g, y):
            zero_fill(dk_hbm, dk_sem, (layer * n_group + g) * step_fill, step_fill)
            heads = _block(g, rep * dh)
            blk = _block(g * _LAYERS + layer, rows)
            q = own_head(_dot(hb, wq_v[:, heads]))
            q_v[blk, :] = q

            def scores(c, m):
                keys = _block(c, _KEYS)
                s = per_batch(q, k_v, g, keys, _NT) * scale
                p_v[blk, keys] = s
                return jnp.maximum(m, _fold_lanes(s, jnp.maximum))

            m = lax.fori_loop(0, win // _KEYS, scores, zero_tile - jnp.inf)
            m = jnp.max(m, axis=-1, keepdims=True)
            e = jnp.exp(p_v[blk, :] - m)
            p_v[blk, :] = e / jnp.sum(e, axis=-1, keepdims=True)

            def values(c, o):
                keys = _block(c, _KEYS)
                return o + per_batch(p_v[blk, keys], v_v, g, keys, _NN)

            o = spread_heads(lax.fori_loop(0, win // _KEYS, values, zero_tile))
            o_v[saved, heads] = o
            return y + _dot(o.astype(_BF16), wo_v[heads, :])

        return x + sum_heads(lax.fori_loop(0, n_group, group, zero_token))

    def attn_bwd(dy, layer):
        saved = _block(layer, rows)
        dya_v[saved, :] = dy
        dyb = dy.astype(_BF16)

        def group(g, dhid):
            done = (_LAYERS + layer) * n_group + g
            zero_fill(dk_hbm, dk_sem, done * step_fill, step_fill)
            heads = _block(g, rep * dh)
            blk = _block(g * _LAYERS + layer, rows)
            do = own_head(_dot(dyb, wo_v[heads, :], _NT))
            do_v[blk, :] = do

            def probs(c, acc):
                keys = _block(c, _KEYS)
                dp = per_batch(do, v_v, g, keys, _NT)
                ds_v[blk, keys] = dp
                return acc + _fold_lanes(dp * p_v[blk, keys], jnp.add)

            delta = lax.fori_loop(0, win // _KEYS, probs, zero_tile)
            delta = jnp.sum(delta, axis=-1, keepdims=True)

            def queries(c, dq):
                keys = _block(c, _KEYS)
                ds = p_v[blk, keys] * (ds_v[blk, keys] - delta) * scale
                ds_v[blk, keys] = ds
                return dq + per_batch(ds, k_v, g, keys, _NN)

            dq = spread_heads(lax.fori_loop(0, win // _KEYS, queries, zero_tile))
            dq_v[saved, heads] = dq
            return dhid + _dot(dq.astype(_BF16), wq_v[:, heads], _NT)

        dhid = sum_heads(lax.fori_loop(0, n_group, group, zero_token))
        return dy + _layernorm_bwd(dhid, ha_v[saved, :], ra_v[saved, 0:1])

    def mlp_fwd(x, layer):
        saved = _block(layer, rows)
        h, rstd = _layernorm(x)
        hm_v[saved, :] = h
        rm_v[saved, :] = jnp.broadcast_to(rstd, (rows, dh))
        hb = h.astype(_BF16)

        def step(c, y):
            units = _block(c, _HIDDEN)
            a, da_du = _gelu_and_grad(_dot(hb, w1_v[:, units]) + bias_v[:, units])
            a_v[saved, units] = a
            dadu_v[saved, units] = da_du
            return y + _dot(a.astype(_BF16), w2_v[units, :])

        y = lax.fori_loop(0, d_ff // _HIDDEN, step, zero_token)
        return x + y + b2_v[...].astype(_F32).reshape(1, d_model)

    def mlp_bwd(dy, layer):
        saved = _block(layer, rows)
        dym_v[saved, :] = once_per_token(dy)
        dyb = dy.astype(_BF16)

        def step(c, dhid):
            units = _block(c, _HIDDEN)
            du = _dot(dyb, w2_v[units, :], _NT) * dadu_v[saved, units]
            du_v[saved, units] = once_per_token(du)
            return dhid + _dot(du.astype(_BF16), w1_v[:, units], _NT)

        dhid = lax.fori_loop(0, d_ff // _HIDDEN, step, zero_token)
        return dy + _layernorm_bwd(dhid, hm_v[saved, :], rm_v[saved, 0:1])

    def forward(layer, x):
        return mlp_fwd(attn_fwd(x, layer), layer)

    def backward(i, dy):
        layer = _LAYERS - 1 - i
        return attn_bwd(mlp_bwd(dy, layer), layer)

    out = lax.fori_loop(0, _LAYERS, forward, tokens(x_v))
    gx = lax.fori_loop(0, _LAYERS, backward, tokens(g_v))
    out_v[...] = untokens(out).astype(out_v.dtype)
    gx_v[...] = untokens(gx).astype(gx_v.dtype)
    db1_v[...] = jnp.sum(du_v[...], axis=0).astype(db1_v.dtype)
    db2_v[...] = jnp.sum(dym_v[...], axis=0).astype(db2_v.dtype)

    def weight_grad(lhs, rhs, ref, tile_rows, tile_cols):
        n_col = ref.shape[1] // tile_cols

        def tile(i):
            r, c = _block(i // n_col, tile_rows), _block(i % n_col, tile_cols)
            ref[r, c] = _dot(
                lhs[:, r].T.astype(_BF16), rhs[:, c].astype(_BF16)
            ).astype(ref.dtype)

        _loop((ref.shape[0] // tile_rows) * n_col, tile)

    weights = (
        (ha_v, dq_v, dwq_v, 128, 2048),
        (o_v, dya_v, dwo_v, 512, d_model),
        (hm_v, du_v, dw1_v, 128, d_ff),
        (a_v, dym_v, dw2_v, _HIDDEN, d_model),
    )
    for i, operands in enumerate(weights):
        zero_fill(dv_hbm, dv_sem, (1 + i) * per_slab, per_slab)
        weight_grad(*operands)

    srow = lax.broadcasted_iota(jnp.int32, (q_v.shape[0], 1), 0)
    slab_of_row = (srow % rows) // rep * n_group + srow // (_LAYERS * rows)

    def mask_slab(s):
        for src, dst in ((q_v, qm_v), (do_v, dom_v)):
            dst[:, _block(s, dh)] = jnp.where(
                slab_of_row == s, src[...], 0.0
            ).astype(dst.dtype)

    _loop(n_slab, mask_slab)
    n_step = win // _GRAD_KEYS
    filled = (1 + len(weights)) * per_slab
    grad_fill = (n_slab // 2) * per_slab // n_step

    def cache_grad(c):
        zero_fill(dv_hbm, dv_sem, filled + c * grad_fill, grad_fill)
        keys = _block(c, _GRAD_KEYS)
        for lhs, rhs, ref in ((ds_v, qm_v, dk_v), (p_v, dom_v, dv_v)):
            res = _dot(lhs[:, keys].T.astype(_BF16), rhs[...])
            for s in range(n_slab):
                ref[s, keys, :] = res[:, s * dh:(s + 1) * dh].astype(ref.dtype)

    _loop(n_step, cache_grad)
    filled += n_step * grad_fill
    zero_fill(dv_hbm, dv_sem, filled, n_slab * per_slab - filled)

    def store_window(src, dst, sem):
        def start(i):
            slabs = _block(i // (win // _GRAD_ROWS), _GRAD_SLABS)
            keys = _block(i % (win // _GRAD_ROWS), _GRAD_ROWS)
            pltpu.make_async_copy(
                src.at[slabs, keys], dst.at[slabs, last, keys], sem
            ).start()

        _loop((n_slab // _GRAD_SLABS) * (win // _GRAD_ROWS), start)

    def store_weight(src, dst, sem):
        per_stream = src.shape[0] // (_WEIGHT_STREAMS * 16)
        width = max(w for w in range(128, 513, 128) if src.shape[1] % w == 0)
        n_col = src.shape[1] // width

        def start(i):
            c = _block(i % n_col, width)
            for stream in range(_WEIGHT_STREAMS):
                r = _block(stream * per_stream + i // n_col, 16)
                pltpu.make_async_copy(src.at[r, c], dst.at[r, c], sem).start()

        _loop(per_stream * n_col, start)

    small = [
        pltpu.make_async_copy(src, dst, out_sem)
        for src, dst in ((out_v, out_hbm), (gx_v, gx_hbm), (db1_v, db1_hbm),
                         (db2_v, db2_hbm))
    ]
    large = ((dwq_v, dwq_hbm), (dwo_v, dwo_hbm), (dw1_v, dw1_hbm),
             (dw2_v, dw2_hbm))
    for cp in small:
        cp.start()
    for i, (src, dst) in enumerate(large):
        store_weight(src, dst, dw_sem.at[i])
    store_window(dk_v, dk_hbm, dk_sem)
    store_window(dv_v, dv_hbm, dv_sem)

    for cp in small:
        cp.wait()
    for i, (src, dst) in enumerate(large):
        pltpu.make_async_copy(src, dst, dw_sem.at[i]).wait()
    pltpu.make_async_copy(dk_hbm, dk_hbm, dk_sem).wait()
    pltpu.make_async_copy(dv_hbm, dv_hbm, dv_sem).wait()


@jax.jit
def pallas_interleave_layers__sliding_block_cached__dense_activation_gelu__decode_kernel(
    A_x: jax.Array,
    A_k_cache: jax.Array,
    A_v_cache: jax.Array,
    A_wq: jax.Array,
    A_wo: jax.Array,
    B_x: jax.Array,
    B_w1: jax.Array,
    B_b1: jax.Array,
    B_w2: jax.Array,
    B_b2: jax.Array,
    grad_out: jax.Array,
):
    del B_x
    n_batch, n_group, seq, dh = A_k_cache.shape
    d_model, d_ff = B_w1.shape
    win = min(4096, max(256, seq // 4))
    rows = n_batch * (_HQ // n_group)
    assert n_batch == 2 and rows == 8 and dh == 128 and seq % win == 0
    n_slab = n_batch * n_group
    stacked = n_group * _LAYERS * rows
    saved = _LAYERS * rows

    parts = (n_slab, seq // win, win, dh)
    x = A_x.reshape(n_batch, d_model)
    inputs = (x, A_k_cache.reshape(parts), A_v_cache.reshape(parts), A_wq, A_wo,
              B_w1, B_b1, B_w2, B_b2, grad_out.reshape(x.shape))
    like = (x, x) + inputs[1:9]

    def staged(arrays):
        return [pltpu.VMEM((n_slab, win, dh) if a.shape == parts else a.shape, a.dtype)
                for a in arrays]

    hbm = pl.BlockSpec(memory_space=pl.ANY)
    res = pl.pallas_call(
        _kernel,
        out_shape=[jax.ShapeDtypeStruct(a.shape, a.dtype) for a in like],
        in_specs=[hbm] * len(inputs),
        out_specs=[hbm] * len(like),
        scratch_shapes=staged(inputs) + staged(like) + [
            pltpu.VMEM((parts[1] - 1, _ZERO_ROWS, dh), A_k_cache.dtype),
            pltpu.VMEM((stacked, win), _F32),
            pltpu.VMEM((stacked, win), _F32),
            pltpu.VMEM((stacked, dh), _F32),
            pltpu.VMEM((stacked, dh), _F32),
            pltpu.VMEM((stacked, n_slab * dh), _BF16),
            pltpu.VMEM((stacked, n_slab * dh), _BF16),
            pltpu.VMEM((saved, d_model), _F32),
            pltpu.VMEM((saved, d_model), _F32),
            pltpu.VMEM((saved, dh), _F32),
            pltpu.VMEM((saved, dh), _F32),
            pltpu.VMEM((saved, _HQ * dh), _F32),
            pltpu.VMEM((saved, _HQ * dh), _F32),
            pltpu.VMEM((saved, d_model), _F32),
            pltpu.VMEM((saved, d_model), _F32),
            pltpu.VMEM((saved, d_ff), _F32),
            pltpu.VMEM((saved, d_ff), _F32),
            pltpu.VMEM((saved, d_ff), _F32),
            pltpu.VMEM((rows, d_ff), _F32),
        ] + [pltpu.SemaphoreType.DMA(())] * 7 + [pltpu.SemaphoreType.DMA((4,))],
        compiler_params=pltpu.CompilerParams(vmem_limit_bytes=112 * 1024 * 1024),
    )(*inputs)
    shaped = (A_x, A_x, A_k_cache, A_v_cache)
    return (*(r.reshape(a.shape) for r, a in zip(res, shaped)), *res[4:])
```
